```python
import os as _os
_os.environ.setdefault("JAX_PLATFORMS", "cpu")
import jax
import jax.numpy as jnp

def _softmax(x, axis=-1):
    return jax.nn.softmax(x, axis=axis)
def _gelu(x):
    return jax.nn.gelu(x, approximate=True)
def _silu(x):
    return jax.nn.silu(x)
def _sigmoid(x):
    return jax.nn.sigmoid(x)
def _layernorm(x, axis=-1, eps=1e-5):
    m = jnp.mean(x, axis=axis, keepdims=True)
    v = jnp.var(x, axis=axis, keepdims=True)
    return (x - m) / jnp.sqrt(v + eps)
def _scatter_add(tgt, idx, src, axis=0):
    return tgt.at[idx].add(src)
def _segment_sum(src, seg, n):
    return jax.ops.segment_sum(src, seg, n)
class _Rng:
    def __init__(self, key):
        self._k = key
    def _next(self):
        self._k, sub = jax.random.split(self._k)
        return sub
    def normal(self, shape):
        return jax.random.normal(self._next(), shape, dtype=jnp.bfloat16)
    def randint(self, lo, hi, shape):
        return jax.random.randint(self._next(), shape, lo, hi, dtype=jnp.int32)
    def uniform(self, shape, lo=0.0, hi=1.0):
        return jax.random.uniform(self._next(), shape, jnp.bfloat16, lo, hi)
    def permutation(self, n):
        return jax.random.permutation(self._next(), n)


kernel_name = 'gated_mix__mha_block__ssm_conv_h3__prompt'

def setup_inputs():
    _rng = _Rng(jax.random.key(int.from_bytes(__import__("os").urandom(4), "little")))
    _w = (lambda a: (lambda t: t.astype(jnp.bfloat16) if jnp.issubdtype(t.dtype, jnp.floating) else t)(jnp.asarray(a)))
    def _A_setup():
        B, S, D, H = 1, 2048, 640, 32
        return {
            "x": _w((lambda *s: _rng.normal(s) * 0.05)(B, S, D)),
            "wqkv": _w((lambda *s: _rng.normal(s) * 0.4)(D, 3 * D)),
            "wo": _w((lambda *s: _rng.normal(s) * 0.05)(D, D)),
        }
    _A_in = _A_setup()

    def _B_setup():
        B, S, D = 1, 2048, 640
        ks = 4
        return {
            "q": _w((lambda *s: _rng.normal(s) * 0.05)(B, S, D)),
            "k": _w((lambda *s: _rng.normal(s) * 0.4)(B, S, D)),
            "v": _w((lambda *s: _rng.normal(s) * 0.4)(B, S, D)),
            "shift_k": _w((lambda *s: _rng.normal(s) * 0.4)(D, ks) * 0.5),
            "ssm_k": _w((lambda *s: _rng.normal(s) * 0.4)(D, S) * (1.0 / S ** 0.5)),
            "ssm_D": _w((lambda *s: _rng.normal(s) * 0.4)(D)),
        }
    _B_in = _B_setup()

    return {
        "A_x": _A_in["x"],
        "A_wqkv": _A_in["wqkv"],
        "A_wo": _A_in["wo"],
        "B_q": _B_in["q"],
        "B_k": _B_in["k"],
        "B_v": _B_in["v"],
        "B_shift_k": _B_in["shift_k"],
        "B_ssm_k": _B_in["ssm_k"],
        "B_ssm_D": _B_in["ssm_D"],
        "gate_w": _w((lambda *s: _rng.normal(s) * 0.05)(640) * 16.0),
    }

def reference(A_x, A_wqkv, A_wo, B_q, B_k, B_v, B_shift_k, B_ssm_k, B_ssm_D, gate_w):
    def _A_ref(x, wqkv, wo):
        B, S, D = x.shape
        H = 32
        Dh = D // H
        qkv = (lambda x, *d: x.transpose(*d))((x @ wqkv).reshape(B, S, 3, H, Dh), 2, 0, 3, 1, 4)
        q, k, v = qkv[0], qkv[1], qkv[2]
        scores = jnp.einsum("bhqd,bhkd->bhqk", q, k) * (Dh ** -0.5)
        p = _softmax(scores, axis=-1)
        o = jnp.einsum("bhqk,bhkd->bhqd", p, v)
        return (lambda x, *d: x.transpose(*d))(o, 0, 2, 1, 3).reshape(B, S, D) @ wo

    def _B_ref(q, k, v, shift_k, ssm_k, ssm_D):
        B, S, D = q.shape
        ks = shift_k.shape[-1]
        k_pad = jnp.pad(k, ((0, 0), (ks - 1, 0), (0, 0)))
        k_shift = jnp.zeros_like(k)
        for t in range(ks):
            k_shift = k_shift + k_pad[:, t:t + S, :] * shift_k[:, ks - 1 - t][None, None, :]
        kv = k_shift * v
        L = 2 * S
        kv_pad = jnp.pad(kv, ((0, 0), (0, S), (0, 0)))
        kf_pad = jnp.pad(ssm_k, ((0, 0), (0, S)))
        kv_f = (lambda x, axes=(-2,-1): jnp.fft.rfft2(x.astype(jnp.float32), axes=axes))(kv_pad[:, None, :, :], axes=(1, 2))
        kf_f = (lambda x, axes=(-2,-1): jnp.fft.rfft2(x.astype(jnp.float32), axes=axes))(kf_pad[:, None, :], axes=(1, 2))
        kf_f = (lambda x, *d: x.transpose(*d))(kf_f, 1, 2, 0)
        y_f = kv_f * kf_f[None, :, :, :]
        y = (lambda x, s, axes=(-2,-1): jnp.fft.irfft2(x, s=s, axes=axes).astype(jnp.bfloat16))(y_f, (1, L), axes=(1, 2))[:, 0, :S, :]
        y = y + kv * ssm_D[None, None, :]
        return q * y

    x = A_x
    g = _sigmoid((x * gate_w).sum(-1, keepdims=True))
    a = _A_ref(x, A_wqkv, A_wo)
    b = _B_ref(x, B_k, B_v, B_shift_k, B_ssm_k, B_ssm_D)
    return g * a + (1 - g) * b
```

```python
import math

import jax
import jax.numpy as jnp
import jax.experimental.pallas as pl
import jax.experimental.pallas.tpu as pltpu

S = 2048
D = 640
H = 32
DH = D // H
KS = 4
L = 128
NT = D // L
NB = S // L
NG = L // 8
VR = 24
TQ = 512
TK = 128
NQB = S // TQ
NKB = S // TK
LAG = 3
CH = 512
NC = S // CH
FB = 512
MG = 8

F32 = jnp.float32
BF16 = jnp.bfloat16
U32 = jnp.uint32
_NT_DIMS = (((1,), (1,)), ((), ()))


def _head_geometry(h):
    lo, hi = DH * h, DH * h + DH - 1
    t0, t1 = lo // L, hi // L
    return t0, t1, lo - L * t0, hi + 1 - L * t1


def _pack(x):
    return pltpu.bitcast(x.astype(BF16), U32)


def _unpack(x):
    return pltpu.bitcast(x, BF16)


def _halves(w):
    return [pltpu.unpack_elementwise(w, index=i, packed_dtype=BF16, unpacked_dtype=F32)
            for i in range(2)]


def _dft_tables():
    def phase(fi, ti):
        f = jnp.where(fi < L // 2, 2 * fi, 2 * fi - (L - 1))
        return ((2 * f + 1) * ti) & (4 * L - 1)

    r = jax.lax.broadcasted_iota(jnp.int32, (2 * L, L), 0)
    n = jax.lax.broadcasted_iota(jnp.int32, (2 * L, L), 1)
    k = phase(r & (L - 1), n) + jnp.where(r >= L, L, 0)
    fwd = jnp.cos(k.astype(F32) * (math.pi / (2 * L))).astype(BF16)
    a = jax.lax.broadcasted_iota(jnp.int32, (L, 2 * L), 0)
    c = jax.lax.broadcasted_iota(jnp.int32, (L, 2 * L), 1)
    k = phase(c >> 1, a) + (c & 1) * L
    inv = (jnp.cos(k.astype(F32) * (math.pi / (2 * L))) * (1.0 / L)).astype(BF16)
    return fwd, inv


def _kernel(x_hbm, wqkv_hbm, wo_hbm, k_hbm, v_hbm, sk_hbm, h_hbm, sd_hbm, gw_hbm,
            o_hbm,
            x_ref, wqkv_ref, wo_ref, k_ref, v_ref, sk_ref, h_ref, sd_ref, gw_ref, o_ref,
            qm_ref, kt_ref, vt_ref, ot_ref, u_ref, hf_ref, hp_ref, z_ref, kv_ref,
            fwd_ref, inv_ref, row_ref, cs_ref, cm_ref, ca_ref,
            wsem, csem, osem):
    def w_copy(i):
        cols = slice(i * D, (i + 1) * D)
        return pltpu.make_async_copy(wqkv_hbm.at[:, cols], wqkv_ref.at[:, cols], wsem.at[i])

    def wo_copy():
        return pltpu.make_async_copy(wo_hbm, wo_ref, wsem.at[3])

    def small_copies():
        return [pltpu.make_async_copy(sk_hbm, sk_ref, wsem.at[4]),
                pltpu.make_async_copy(sd_hbm, sd_ref, wsem.at[5]),
                pltpu.make_async_copy(gw_hbm, gw_ref, wsem.at[6])]

    def x_copy(c):
        rows = pl.ds(pl.multiple_of(c * CH, CH), CH)
        return pltpu.make_async_copy(x_hbm.at[rows, :], x_ref.at[rows, :], csem.at[c])

    def conv_copies(c):
        rows = pl.ds(pl.multiple_of(c * CH, CH), CH)
        krows = pl.ds(pl.multiple_of(c * CH + 16, 16), CH)
        return [
            pltpu.make_async_copy(k_hbm.at[rows, :], k_ref.at[krows, :], csem.at[NC + c]),
            pltpu.make_async_copy(v_hbm.at[rows, :], v_ref.at[rows, :], csem.at[2 * NC + c]),
            pltpu.make_async_copy(h_hbm.at[:, rows], h_ref.at[:, rows], csem.at[3 * NC + c]),
        ]

    def out_copy(i):
        rows = slice(i * L, (i + 1) * L)
        return pltpu.make_async_copy(o_ref.at[rows, :], o_hbm.at[rows, :], osem.at[i])

    x_copy(0).start()
    w_copy(0).start()

    lane = jax.lax.broadcasted_iota(jnp.int32, (1, L), 1)
    row8 = jax.lax.broadcasted_iota(jnp.int32, (8, 1), 0)
    qscale = (DH ** -0.5) * math.log2(math.e)

    def chunk_rows(c):
        return (pl.ds(pl.multiple_of(c * CH, CH), CH),
                pl.ds(pl.multiple_of(c * (CH // 2), CH // 2), CH // 2))

    def proj_q(c):
        rows, prows = chunk_rows(c)
        q = jnp.dot(x_ref[rows, :], wqkv_ref[:, 0:D], preferred_element_type=F32)
        qt = [_pack(q[:, t * L:(t + 1) * L] * qscale) for t in range(NT)]
        zero = jnp.uint32(0)
        for h in range(H):
            t0, t1, lo, hi = _head_geometry(h)
            if t0 == t1:
                qm = jnp.where((lane >= lo) & (lane < hi), qt[t0], zero)
            else:
                qm = jnp.where(lane >= lo, qt[t0], jnp.where(lane < hi, qt[t1], zero))
            qm_ref[h, prows, :] = qm

    def proj_k(c):
        rows, prows = chunk_rows(c)
        k = jnp.dot(x_ref[rows, :], wqkv_ref[:, D:2 * D], preferred_element_type=F32)
        kt = [_pack(k[:, t * L:(t + 1) * L]) for t in range(NT)]
        for t in range(NT):
            kt_ref[t, prows, :] = kt[t]
        for t in range(NT - 1):
            kt_ref[NT + t, prows, :] = jnp.where(lane >= L // 2, kt[t], kt[t + 1])

    def proj_v(c):
        rows, _ = chunk_rows(c)
        v = jnp.dot(x_ref[rows, :], wqkv_ref[:, 2 * D:3 * D], preferred_element_type=F32)
        vt = v.astype(BF16).astype(F32).T
        for p in range(H // 2):
            b = 2 * DH * p
            mid = vt[b + 16:b + 24]
            vt_ref[2 * p, 0:16, rows] = vt[b:b + 16]
            vt_ref[2 * p, 16:24, rows] = jnp.where(row8 == 4, 1.0, mid)
            vt_ref[2 * p + 1, 0:8, rows] = jnp.where(row8 == 0, 1.0, mid)
            vt_ref[2 * p + 1, 8:24, rows] = vt[b + 24:b + 40]

    def conv_u(j):
        b0 = pl.multiple_of(j * L, L)
        for t in range(NT):
            cs = slice(t * L, (t + 1) * L)
            w = pltpu.bitcast(k_ref[pl.ds(b0, L + 16), cs], U32)
            e0, o0 = _halves(w[8:8 + L // 2])
            e1, o1 = _halves(pltpu.roll(w, 1, 0)[8:8 + L // 2])
            o2 = _halves(pltpu.roll(w, 2, 0)[8:8 + L // 2])[1]
            s0, s1, s2, s3 = [row_ref[d:d + 1, cs] for d in range(KS)]
            ve, vo = _halves(pltpu.bitcast(v_ref[pl.ds(b0, L), cs], U32))
            kve = (e0 * s0 + o1 * s1 + e1 * s2 + o2 * s3) * ve
            kvo = (o0 * s0 + e0 * s1 + o1 * s2 + e1 * s3) * vo
            kv = pltpu.pack_elementwise([kve, kvo], packed_dtype=BF16)
            kv_ref[t, pl.ds(pl.multiple_of(j * (L // 2), L // 2), L // 2), :] = kv
            u = jnp.dot(fwd_ref[...], _unpack(kv), preferred_element_type=F32)
            for c in range(2):
                u_ref[:, t, j, c] = u[c * L:(c + 1) * L].reshape(NG, 8, L)

    def conv_h(j, hp):
        b0 = pl.multiple_of(j * L, L)
        hc = jax.lax.dot_general(fwd_ref[...], h_ref[:, pl.ds(b0, L)],
                                 _NT_DIMS, preferred_element_type=F32)
        hl = L // 2
        hf = jnp.concatenate([
            hc[0:hl] - hp[L:L + hl], hc[hl:L] + hp[L + hl:2 * L],
            hc[L:L + hl] + hp[0:hl], hc[L + hl:2 * L] - hp[hl:L]], axis=0)
        for t in range(NT):
            for c in range(2):
                hf_ref[:, t, j, c] = (
                    hf[c * L:(c + 1) * L, t * L:(t + 1) * L].reshape(NG, 8, L))
        return hc

    fwd, inv = _dft_tables()
    fwd_ref[...] = fwd
    inv_ref[...] = inv
    hp_ref[...] = jnp.zeros(hp_ref.shape, F32)
    k_ref[0:16, :] = jnp.zeros((16, D), BF16)
    cs_ref[...] = jnp.zeros(cs_ref.shape, F32)
    cm_ref[...] = jnp.zeros(cm_ref.shape, F32)
    ca_ref[...] = jnp.ones(ca_ref.shape, F32)

    w_copy(0).wait()
    for c in range(1, NC):
        x_copy(c).start()

    def qpass(c, carry):
        x_copy(c).wait()

        @pl.when(c == 1)
        def _():
            for cp in [w_copy(1), w_copy(2)] + small_copies() + conv_copies(0):
                cp.start()

        proj_q(c)
        return carry

    jax.lax.fori_loop(0, NC, qpass, 0)
    for c in range(1, NC):
        for cp in conv_copies(c):
            cp.start()
    wo_copy().start()
    for cp in [w_copy(1), w_copy(2)] + small_copies():
        cp.wait()
    row_ref[0:KS, :] = sk_ref[...].astype(F32)
    for t in range(NT):
        row_ref[KS:KS + 1, t * L:(t + 1) * L] = sd_ref[...].astype(F32)[t:t + 1]
        row_ref[KS + 1:KS + 2, t * L:(t + 1) * L] = gw_ref[...].astype(F32)[t:t + 1]

    def kvpass(c, carry):
        for cp in conv_copies(c):
            cp.wait()
        proj_v(c)
        hp = hp_ref[...]
        for s in range(CH // L):
            j = c * (CH // L) + s
            hp = conv_h(j, hp)
            conv_u(j)
        hp_ref[...] = hp
        proj_k(c)
        return carry

    jax.lax.fori_loop(0, NC, kvpass, 0)
    wo_copy().wait()

    def ktile(h):
        lo = h * DH
        t0 = lo // L
        return t0 + NT * ((lo - t0 * L) > (L - DH)).astype(jnp.int32)

    def attention(p, flush_only=False):
        heads = {0: 2 * p, 1: 2 * p + 1,
                 -1: H - 1 if flush_only else jnp.maximum(2 * p - 1, 0)}
        blocks = [(-1, NQB - 1, kb) for kb in range(NKB - LAG, NKB)]
        if not flush_only:
            kidx = [ktile(heads[e]) for e in range(2)]
            blocks += [(e, qi, kb) for qi in range(NQB) for e in range(2)
                       for kb in range(NKB)]
        ss = {blocks[n]: cs_ref[n] for n in range(LAG)}
        ms = {(-1, NQB - 1): cm_ref[0:1]}
        accs = {(-1, NQB - 1): ca_ref[0]}
        outs = {(-2, NQB - 1): ca_ref[1]}

        def qk(e, qi, kb):
            q = _unpack(qm_ref[heads[e], qi * TQ // 2:(qi + 1) * TQ // 2, :])
            kk = _unpack(kt_ref[kidx[e], kb * TK // 2:(kb + 1) * TK // 2, :])
            ss[(e, qi, kb)] = jax.lax.dot_general(kk, q, _NT_DIMS,
                                                  preferred_element_type=F32)

        def softmax_pv(e, qi, kb):
            st = ss.pop((e, qi, kb))
            mn = jnp.max(st, axis=0, keepdims=True)
            if kb > 0:
                mn = jnp.maximum(ms[(e, qi)], mn)
                alpha = jnp.exp2(ms[(e, qi)] - mn)
            ms[(e, qi)] = mn
            pt = jnp.exp2(st - mn).astype(BF16)
            r = jnp.dot(vt_ref[heads[e], :, kb * TK:(kb + 1) * TK], pt,
                        preferred_element_type=F32)
            accs[(e, qi)] = r if kb == 0 else accs[(e, qi)] * alpha + r
            if kb == NKB - 1:
                acc = accs.pop((e, qi))
                den = acc[20:21] if e % 2 == 0 else acc[0:1]
                outs[(e, qi)] = acc * (1.0 / den)
                if e % 2 == 1:
                    oe, oo = outs.pop((e - 1, qi)), outs.pop((e, qi))
                    cols = slice(qi * TQ, (qi + 1) * TQ)
                    slot = p + e // 2 + 1
                    ot_ref[slot, 0:16, cols] = oe[0:16]
                    ot_ref[slot, 16:24, cols] = jnp.where(row8 < 4, oe[16:24], oo[0:8])
                    ot_ref[slot, 24:40, cols] = oo[8:24]

        if flush_only:
            for b in blocks:
                softmax_pv(*b)
            return

        zacc = {}

        def conv_step(t, i0, m, zero):
            hr, hi_ = hf_ref[p, t, m, 0] + zero, hf_ref[p, t, m, 1] + zero
            for i in range(max(i0, m), i0 + MG):
                ur, ui = u_ref[p, t, i - m, 0], u_ref[p, t, i - m, 1]
                tr = ur * hr - ui * hi_
                ti = ur * hi_ + ui * hr
                if m > 0:
                    tr, ti = zacc[i][0] + tr, zacc[i][1] + ti
                zacc[i] = (tr, ti)
                if m == i:
                    z_ref[i, t, p] = pltpu.pack_elementwise([tr, ti], packed_dtype=BF16)

        steps = [(t, i0, m) for t in range(NT) for i0 in range(0, NB, MG)
                 for m in range(i0 + MG)]
        nb = len(blocks) - LAG
        for n in range(nb):
            qk(*blocks[n + LAG])
            softmax_pv(*blocks[n])
            zero = jnp.where(ms[blocks[n][:2]][:, 0:L] > 0, 0.0, -0.0)
            for step in steps[n * len(steps) // nb:(n + 1) * len(steps) // nb]:
                conv_step(*step, zero)
        for n in range(LAG):
            cs_ref[n] = ss.pop(blocks[nb + n])
        cm_ref[0:1] = ms[(1, NQB - 1)]
        ca_ref[0] = accs.pop((1, NQB - 1))
        ca_ref[1] = outs.pop((0, NQB - 1))

    def pair(p, carry):
        attention(p)
        return carry

    jax.lax.fori_loop(0, H // 2, pair, 0)
    attention(H // 2, flush_only=True)

    for c in range(S // FB):
        ot = ot_ref[1:, :, c * FB:(c + 1) * FB].reshape(D, FB)
        a_all = jnp.dot(ot.T.astype(BF16), wo_ref[...], preferred_element_type=F32)
        for s in range(FB // L):
            i = c * (FB // L) + s
            rows = slice(i * L, (i + 1) * L)
            prows = slice(i * L // 2, (i + 1) * L // 2)
            w = jnp.concatenate(
                [_unpack(z_ref[i, t].reshape(L, L)) for t in range(NT)], axis=1)
            y = jnp.dot(inv_ref[...], w, preferred_element_type=F32)
            a = a_all[s * L:(s + 1) * L]
            x = x_ref[rows, :].astype(F32)
            kv = jnp.concatenate(
                [_unpack(kv_ref[t, prows, :]) for t in range(NT)], axis=1).astype(F32)
            g = jax.nn.sigmoid(
                jnp.sum(x * row_ref[KS + 1:KS + 2, :], axis=-1, keepdims=True))
            b = x * (y + kv * row_ref[KS:KS + 1, :])
            o_ref[rows, :] = (g * a + (1.0 - g) * b).astype(o_ref.dtype)
            out_copy(i).start()
    for i in range(NB):
        out_copy(i).wait()


@jax.jit
def pallas_gated_mix__mha_block__ssm_conv_h3__prompt_kernel(
    A_x: jax.Array,
    A_wqkv: jax.Array,
    A_wo: jax.Array,
    B_q: jax.Array,
    B_k: jax.Array,
    B_v: jax.Array,
    B_shift_k: jax.Array,
    B_ssm_k: jax.Array,
    B_ssm_D: jax.Array,
    gate_w: jax.Array,
):
    del B_q
    out = pl.pallas_call(
        _kernel,
        out_shape=jax.ShapeDtypeStruct((S, D), BF16),
        in_specs=[pl.BlockSpec(memory_space=pl.ANY)] * 9,
        out_specs=pl.BlockSpec(memory_space=pl.ANY),
        scratch_shapes=[
            pltpu.VMEM((S, D), BF16),
            pltpu.VMEM((D, 3 * D), BF16),
            pltpu.VMEM((D, D), BF16),
            pltpu.VMEM((S + 16, D), BF16),
            pltpu.VMEM((S, D), BF16),
            pltpu.VMEM((KS, D), BF16),
            pltpu.VMEM((D, S), BF16),
            pltpu.VMEM((NT, L), BF16),
            pltpu.VMEM((NT, L), BF16),
            pltpu.VMEM((S, D), BF16),
            pltpu.VMEM((H, S // 2, L), U32),
            pltpu.VMEM((2 * NT - 1, S // 2, L), U32),
            pltpu.VMEM((H, VR, S), F32),
            pltpu.VMEM((H // 2 + 1, 2 * DH, S), F32),
            pltpu.VMEM((NG, NT, NB, 2, 8, L), F32),
            pltpu.VMEM((NG, NT, NB, 2, 8, L), F32),
            pltpu.VMEM((2 * L, D), F32),
            pltpu.VMEM((NB, NT, NG, 8, L), U32),
            pltpu.VMEM((NT, S // 2, L), U32),
            pltpu.VMEM((2 * L, L), BF16),
            pltpu.VMEM((L, 2 * L), BF16),
            pltpu.VMEM((8, D), F32),
            pltpu.VMEM((LAG, TK, TQ), F32),
            pltpu.VMEM((8, TQ), F32),
            pltpu.VMEM((2, VR, TQ), F32),
            pltpu.SemaphoreType.DMA((7,)),
            pltpu.SemaphoreType.DMA((4 * NC,)),
            pltpu.SemaphoreType.DMA((NB,)),
        ],
        compiler_params=pltpu.CompilerParams(vmem_limit_bytes=110 * 1024 * 1024),
    )(A_x.reshape(S, D), A_wqkv, A_wo, B_k.reshape(S, D), B_v.reshape(S, D),
      B_shift_k.T, B_ssm_k, B_ssm_D.reshape(NT, L), gate_w.reshape(NT, L))
    return out.reshape(1, S, D)
```

```python
import functools
import math

import jax
import jax.numpy as jnp
import jax.experimental.pallas as pl
import jax.experimental.pallas.tpu as pltpu

S = 2048
D = 640
H = 32
DH = D // H
KS = 4
L = 128
NT = D // L
NB = S // L
NG = L // 8
VR = 24
TQ = 512
TK = 128
NQB = S // TQ
NKB = S // TK
LAG = 3
CH = 512
NC = S // CH
CB = CH // L
QB = (NB - CB) // 2
RA = 2
TA = 3

F32 = jnp.float32
BF16 = jnp.bfloat16
U32 = jnp.uint32
_NT_DIMS = (((1,), (1,)), ((), ()))


def _head_geometry(h):
    lo, hi = DH * h, DH * h + DH - 1
    t0, t1 = lo // L, hi // L
    return t0, t1, lo - L * t0, hi + 1 - L * t1


def _pack(x):
    return pltpu.bitcast(x.astype(BF16), U32)


def _unpack(x):
    return pltpu.bitcast(x, BF16)


def _halves(w):
    return [jax.lax.bitcast_convert_type(w << 16, F32),
            jax.lax.bitcast_convert_type(w & jnp.uint32(0xFFFF0000), F32)]


def _pack_pair(lo, hi):
    def bits(x):
        return jax.lax.bitcast_convert_type(x.astype(BF16).astype(F32), U32)
    return (bits(lo) >> 16) | bits(hi)


def _dft_tables():
    def cos_table(k):
        k = k & (4 * L - 1)
        return jnp.cos(k.astype(F32) * (math.pi / (2 * L)))

    r = jax.lax.broadcasted_iota(jnp.int32, (2 * L, L), 0)
    n = jax.lax.broadcasted_iota(jnp.int32, (2 * L, L), 1)
    fr = r & (L - 1)
    f = jnp.where(fr < L // 2, 2 * fr, 2 * L - 1 - 2 * fr)
    fwd = cos_table((2 * f + 1) * n + jnp.where(r >= L, L, 0))
    a = jax.lax.broadcasted_iota(jnp.int32, (L, L), 0)
    c = jax.lax.broadcasted_iota(jnp.int32, (L, L), 1)
    t = jnp.where(a < L // 2, 2 * a, 2 * a - (L - 1))
    inv = cos_table((4 * (c >> 1) + 1) * t + (c & 1) * L) * (1.0 / L)
    return _pack(fwd), _pack(inv)


def _kernel(x_hbm, wqkv_hbm, wo_hbm, k_hbm, v_hbm, sk_hbm, h_hbm, sd_hbm, gw_hbm,
            o_hbm,
            x_ref, wqkv_ref, wo_ref, k_ref, v_ref, sk_ref, h_ref, sd_ref, gw_ref, o_ref,
            qm_ref, kt_ref, vt_ref, ot_ref, u_ref, hf_ref, hp_ref, z_ref, g_ref,
            fwd_ref, inv_ref, row_ref, cs_ref, cm_ref, ca_ref,
            wsem, csem, osem):
    def w_copy(i):
        cols = slice(i * D, (i + 1) * D)
        return pltpu.make_async_copy(wqkv_hbm.at[:, cols], wqkv_ref.at[:, cols], wsem.at[i])

    def wo_copy():
        return pltpu.make_async_copy(wo_hbm, wo_ref, wsem.at[3])

    def small_copies():
        return [pltpu.make_async_copy(sk_hbm, sk_ref, wsem.at[4]),
                pltpu.make_async_copy(sd_hbm, sd_ref, wsem.at[4]),
                pltpu.make_async_copy(gw_hbm, gw_ref, wsem.at[4])]

    def x_copy(c):
        blk = pl.ds(CB + (c - 1) * QB, QB)
        return pltpu.make_async_copy(x_hbm.at[blk], x_ref.at[blk], csem.at[c])

    def conv_copies(c):
        rows = pl.ds(pl.multiple_of(c * CH, CH), CH)
        blk = pl.ds(c * CB, CB)
        sem = csem.at[3 + c]
        return [pltpu.make_async_copy(k_hbm.at[blk], k_ref.at[pl.ds(c * CB + 1, CB)], sem),
                pltpu.make_async_copy(v_hbm.at[blk], v_ref.at[blk], sem),
                pltpu.make_async_copy(h_hbm.at[:, rows], h_ref.at[c], sem)]

    def out_copy(i):
        rows = slice(i * L, (i + 1) * L)
        return pltpu.make_async_copy(o_ref.at[rows, :], o_hbm.at[rows, :], osem.at[0])

    def first_copies(part):
        blk = slice(0, RA) if part == 0 else slice(RA, CB)
        cols = slice(0, TA * L) if part == 0 else slice(TA * L, D)
        sem = wsem.at[0] if part == 0 else csem.at[0]
        return [pltpu.make_async_copy(x_hbm.at[blk], x_ref.at[blk], sem),
                pltpu.make_async_copy(wqkv_hbm.at[:, cols], wqkv_ref.at[:, cols], sem)]

    for cp in first_copies(0) + first_copies(1):
        cp.start()

    lane = jax.lax.broadcasted_iota(jnp.int32, (1, L), 1)
    row8 = jax.lax.broadcasted_iota(jnp.int32, (8, 1), 0)
    qscale = (DH ** -0.5) * math.log2(math.e)

    def chunk_rows(c):
        return (pl.ds(pl.multiple_of(c * CH, CH), CH),
                pl.ds(pl.multiple_of(c * (CH // 2), CH // 2), CH // 2))

    def x_rows(b0, nb):
        return x_ref[pl.ds(b0, nb)].reshape(nb * L, D)

    def proj_q(b0, nb, t_lo=0, t_hi=NT, qt=None):
        prows = pl.ds(pl.multiple_of(b0 * (L // 2), L // 2), nb * L // 2)
        q = jnp.dot(x_rows(b0, nb), wqkv_ref[:, t_lo * L:t_hi * L],
                    preferred_element_type=F32)
        qt = dict(qt or {})
        for t in range(t_lo, t_hi):
            qt[t] = _pack(q[:, (t - t_lo) * L:(t - t_lo + 1) * L] * qscale)
        zero = jnp.uint32(0)
        for h in range(H):
            t0, t1, lo, hi = _head_geometry(h)
            if not t_lo <= t1 < t_hi:
                continue
            if t0 == t1:
                qm = jnp.where((lane >= lo) & (lane < hi), qt[t0], zero)
            else:
                qm = jnp.where(lane >= lo, qt[t0], jnp.where(lane < hi, qt[t1], zero))
            qm_ref[h, prows, :] = qm
        return qt

    def proj_k(c):
        _, prows = chunk_rows(c)
        k = jnp.dot(x_rows(c * CB, CB), wqkv_ref[:, D:2 * D], preferred_element_type=F32)
        kt = [_pack(k[:, t * L:(t + 1) * L]) for t in range(NT)]
        for t in range(NT):
            kt_ref[t, prows, :] = kt[t]
        for t in range(NT - 1):
            kt_ref[NT + t, prows, :] = jnp.where(lane >= L // 2, kt[t], kt[t + 1])

    def proj_v(c):
        rows, _ = chunk_rows(c)
        v = jnp.dot(x_rows(c * CB, CB), wqkv_ref[:, 2 * D:3 * D], preferred_element_type=F32)
        vt = v.astype(BF16).astype(F32).T
        for p in range(H // 2):
            b = 2 * DH * p
            mid = vt[b + 16:b + 24]
            vt_ref[2 * p, 0:16, rows] = vt[b:b + 16]
            vt_ref[2 * p, 16:24, rows] = jnp.where(row8 == 4, 1.0, mid)
            vt_ref[2 * p + 1, 0:8, rows] = jnp.where(row8 == 0, 1.0, mid)
            vt_ref[2 * p + 1, 8:24, rows] = vt[b + 24:b + 40]

    def conv_u(c, s):
        j = c * CB + s
        for t in range(NT):
            cs = slice(t * L, (t + 1) * L)
            w = jnp.concatenate([pltpu.bitcast(k_ref[j, L - 16:L, cs], U32),
                                 pltpu.bitcast(k_ref[j + 1, :, cs], U32)], axis=0)
            e0, o0 = _halves(w[8:8 + L // 2])
            e1, o1 = _halves(pltpu.roll(w, 1, 0)[8:8 + L // 2])
            o2 = _halves(pltpu.roll(w, 2, 0)[8:8 + L // 2])[1]
            s0, s1, s2, s3 = [row_ref[d:d + 1, cs] for d in range(KS)]
            ve, vo = _halves(pltpu.bitcast(v_ref[j, :, cs], U32))
            kve = (e0 * s0 + o1 * s1 + e1 * s2 + o2 * s3) * ve
            kvo = (o0 * s0 + e0 * s1 + o1 * s2 + e1 * s3) * vo
            u = jnp.dot(_unpack(fwd_ref[...]), _unpack(_pack_pair(kve, kvo)),
                        preferred_element_type=F32)
            for r in range(2):
                u_ref[:, t, c, 2 * s + r] = u[r * L:(r + 1) * L].reshape(NG, 8, L)

    def conv_h(c, s, hp, skip):
        hc = jax.lax.dot_general(_unpack(fwd_ref[...]), h_ref[c, :, s * L:(s + 1) * L],
                                 _NT_DIMS, preferred_element_type=F32)
        if skip is not None:
            hc = jnp.concatenate([hc[0:L] + skip, hc[L:2 * L]], axis=0)
        hl = L // 2
        hf = jnp.concatenate([
            hc[0:hl] - hp[L:L + hl], hc[hl:L] + hp[L + hl:2 * L],
            hc[L:L + hl] + hp[0:hl], hc[L + hl:2 * L] - hp[hl:L]], axis=0)
        for t in range(NT):
            for r in range(2):
                hf_ref[:, t, c, 2 * s + r] = (
                    hf[r * L:(r + 1) * L, t * L:(t + 1) * L].reshape(NG, 8, L))
        return hc

    fwd_ref[...], inv_ref[...] = _dft_tables()
    hp_ref[...] = jnp.zeros(hp_ref.shape, F32)
    k_ref[0, L - 16:L, :] = jnp.zeros((16, D), BF16)
    cs_ref[...] = jnp.zeros(cs_ref.shape, F32)
    cm_ref[...] = jnp.zeros(cm_ref.shape, F32)
    ca_ref[...] = jnp.ones(ca_ref.shape, F32)

    for cp in first_copies(0):
        cp.wait()
    x_copy(1).start()
    qt = [proj_q(b, 1, 0, TA) for b in range(RA)]
    for cp in first_copies(1):
        cp.wait()
    x_copy(2).start()
    proj_q(RA, CB - RA)
    for b in range(RA):
        proj_q(b, 1, TA, NT, qt[b])

    def qpass(c, carry):
        x_copy(c).wait()

        @pl.when(c == 1)
        def _():
            for cp in small_copies() + [w_copy(1), w_copy(2)] + conv_copies(0):
                cp.start()

        proj_q(CB + (c - 1) * QB, QB)
        return carry

    jax.lax.fori_loop(1, 3, qpass, 0)
    for c in range(1, NC):
        for cp in conv_copies(c):
            cp.start()
    wo_copy().start()
    w_copy(1).wait()
    w_copy(2).wait()
    for cp in small_copies():
        cp.wait()
    row_ref[0:KS, :] = sk_ref[...].astype(F32)
    for t in range(NT):
        row_ref[KS:KS + 1, t * L:(t + 1) * L] = sd_ref[...].astype(F32)[t:t + 1]
        row_ref[KS + 1:KS + 2, t * L:(t + 1) * L] = gw_ref[...].astype(F32)[t:t + 1]

    def kvpass(c, carry):
        for cp in conv_copies(c):
            cp.wait()
        proj_v(c)
        hp = hp_ref[...]
        for s in range(CB):
            skip = jnp.where(c == 0, row_ref[KS:KS + 1, :], 0.0) if s == 0 else None
            hp = conv_h(c, s, hp, skip)
            conv_u(c, s)
        hp_ref[...] = hp
        proj_k(c)
        return carry

    jax.lax.fori_loop(0, NC, kvpass, 0)
    wo_copy().wait()

    def ktile(h):
        lo = h * DH
        t0 = lo // L
        return t0 + NT * ((lo - t0 * L) > (L - DH)).astype(jnp.int32)

    def attention(p, flush_only=False):
        heads = {0: 2 * p, 1: 2 * p + 1,
                 -1: H - 1 if flush_only else jnp.maximum(2 * p - 1, 0)}
        blocks = [(-1, NQB - 1, kb) for kb in range(NKB - LAG, NKB)]
        if not flush_only:
            kidx = [ktile(heads[e]) for e in range(2)]
            blocks += [(e, qi, kb) for qi in range(NQB) for e in range(2)
                       for kb in range(NKB)]
        ss = {blocks[n]: cs_ref[n] for n in range(LAG)}
        ms = {(-1, NQB - 1): cm_ref[0:1]}
        accs = {(-1, NQB - 1): ca_ref[0]}
        outs = {(-2, NQB - 1): ca_ref[1]}

        def qk(e, qi, kb):
            q = _unpack(qm_ref[heads[e], qi * TQ // 2:(qi + 1) * TQ // 2, :])
            kk = _unpack(kt_ref[kidx[e], kb * TK // 2:(kb + 1) * TK // 2, :])
            ss[(e, qi, kb)] = jax.lax.dot_general(kk, q, _NT_DIMS,
                                                  preferred_element_type=F32)

        def softmax_pv(e, qi, kb):
            st = ss.pop((e, qi, kb))
            mn = jnp.max(st, axis=0, keepdims=True)
            if kb > 0:
                mn = jnp.maximum(ms[(e, qi)], mn)
                alpha = jnp.exp2(ms[(e, qi)] - mn)
            ms[(e, qi)] = mn
            pt = jnp.exp2(st - mn).astype(BF16)
            r = jnp.dot(vt_ref[heads[e], :, kb * TK:(kb + 1) * TK], pt,
                        preferred_element_type=F32)
            accs[(e, qi)] = r if kb == 0 else accs[(e, qi)] * alpha + r
            if kb == NKB - 1:
                acc = accs.pop((e, qi))
                den = acc[20:21] if e % 2 == 0 else acc[0:1]
                outs[(e, qi)] = acc * (1.0 / den)
                if e % 2 == 1:
                    oe, oo = outs.pop((e - 1, qi)), outs.pop((e, qi))
                    cols = slice(qi * TQ, (qi + 1) * TQ)
                    slot = p + e // 2 + 1
                    ot_ref[slot, 0:16, cols] = oe[0:16]
                    ot_ref[slot, 16:24, cols] = jnp.where(row8 < 4, oe[16:24], oo[0:8])
                    ot_ref[slot, 24:40, cols] = oo[8:24]

        if flush_only:
            return [functools.partial(softmax_pv, *b) for b in blocks]

        zacc = {}
        pz = p & (NG // 2 - 1)
        pq = p ^ (NG // 2)

        def at(g, t, j, r):
            return (g, t, j // CB, 2 * (j % CB) + r)

        def conv_step(t, m, zero):
            hr, hi_ = hf_ref[at(p, t, m, 0)] + zero, hf_ref[at(p, t, m, 1)] + zero
            for i in range(m, NB):
                ur, ui = u_ref[at(p, t, i - m, 0)], u_ref[at(p, t, i - m, 1)]
                tr = ur * hr - ui * hi_
                ti = ur * hi_ + ui * hr
                if m > 0:
                    tr, ti = zacc[i][0] + tr, zacc[i][1] + ti
                zacc[i] = (tr, ti)
                if m == i:
                    wr, wi = hf_ref[at(pq, t, i, 0)], hf_ref[at(pq, t, i, 1)]
                    hf_ref[at(p, t, i, 0)] = tr
                    hf_ref[at(p, t, i, 1)] = ti
                    z_ref[pz, i, 0, t] = _pack_pair(wr + tr, wi - ti)
                    z_ref[pz, i, 1, t] = _pack_pair(wr - tr, wi + ti)

        steps = [(t, m) for t in range(NT) for m in range(NB)]
        nb = len(blocks) - LAG
        hosts = [n for n in range(nb) if blocks[n][2] not in (0, NKB - 1)]
        slot_of = [hosts[k * len(hosts) // len(steps)] for k in range(len(steps))]
        for n in range(nb):
            qk(*blocks[n + LAG])
            softmax_pv(*blocks[n])
            zero = jnp.where(ss[blocks[n + LAG]][0:8, 0:L] > 0, 0.0, -0.0)
            for step, host in zip(steps, slot_of):
                if host == n:
                    conv_step(*step, zero)
        rows = pl.ds(pl.multiple_of(p * L, L), L)
        logit = jnp.sum(x_ref[p].astype(F32) * row_ref[KS + 1:KS + 2, :],
                        axis=-1, keepdims=True)
        g_ref[rows, :] = jnp.broadcast_to(jax.nn.sigmoid(logit), (L, L))
        for n in range(LAG):
            cs_ref[n] = ss.pop(blocks[nb + n])
        cm_ref[0:1] = ms[(1, NQB - 1)]
        ca_ref[0] = accs.pop((1, NQB - 1))
        ca_ref[1] = outs.pop((0, NQB - 1))

    def pair(p, carry):
        attention(p)
        return carry

    jax.lax.fori_loop(0, H // 2, pair, 0)

    flush = attention(H // 2, flush_only=True)
    for i in range(NB):
        rows = slice(i * L, (i + 1) * L)
        yh = []
        for e in range(2):
            w = jnp.concatenate(
                [_unpack(z_ref[:, i, e, t].reshape(L // 2, L)) for t in range(NT)], axis=1)
            yh.append(jnp.dot(_unpack(inv_ref[e * L // 4:(e + 1) * L // 4, :]), w,
                              preferred_element_type=F32))
        y = _unpack(_pack_pair(*yh)).astype(F32)
        b = (jnp.concatenate([1.0 - g_ref[rows, :]] * NT, axis=1)
             * (x_ref[i].astype(F32) * y))
        ot = ot_ref[1:, :, rows].reshape(D, L)
        a = jnp.dot(ot.T.astype(BF16), wo_ref[...], preferred_element_type=F32)
        g = jnp.concatenate([g_ref[rows, :]] * NT, axis=1)
        o_ref[rows, :] = (g * a + b).astype(o_ref.dtype)
        out_copy(i).start()
        if i < LAG:
            flush[i]()
    for i in range(NB):
        out_copy(i).wait()


@jax.jit
def pallas_gated_mix__mha_block__ssm_conv_h3__prompt_kernel(
    A_x: jax.Array,
    A_wqkv: jax.Array,
    A_wo: jax.Array,
    B_q: jax.Array,
    B_k: jax.Array,
    B_v: jax.Array,
    B_shift_k: jax.Array,
    B_ssm_k: jax.Array,
    B_ssm_D: jax.Array,
    gate_w: jax.Array,
):
    del B_q
    out = pl.pallas_call(
        _kernel,
        out_shape=jax.ShapeDtypeStruct((S, D), BF16),
        in_specs=[pl.BlockSpec(memory_space=pl.ANY)] * 9,
        out_specs=pl.BlockSpec(memory_space=pl.ANY),
        scratch_shapes=[
            pltpu.VMEM((NB, L, D), BF16),
            pltpu.VMEM((D, 3 * D), BF16),
            pltpu.VMEM((D, D), BF16),
            pltpu.VMEM((NB + 1, L, D), BF16),
            pltpu.VMEM((NB, L, D), BF16),
            pltpu.VMEM((KS, D), BF16),
            pltpu.VMEM((NC, D, CH), BF16),
            pltpu.VMEM((NT, L), BF16),
            pltpu.VMEM((NT, L), BF16),
            pltpu.VMEM((S, D), BF16),
            pltpu.VMEM((H, S // 2, L), U32),
            pltpu.VMEM((2 * NT - 1, S // 2, L), U32),
            pltpu.VMEM((H, VR, S), F32),
            pltpu.VMEM((H // 2 + 1, 2 * DH, S), F32),
            pltpu.VMEM((NG, NT, NC, 2 * CB, 8, L), F32),
            pltpu.VMEM((NG, NT, NC, 2 * CB, 8, L), F32),
            pltpu.VMEM((2 * L, D), F32),
            pltpu.VMEM((NG // 2, NB, 2, NT, 8, L), U32),
            pltpu.VMEM((S, L), F32),
            pltpu.VMEM((L, L), U32),
            pltpu.VMEM((L // 2, L), U32),
            pltpu.VMEM((8, D), F32),
            pltpu.VMEM((LAG, TK, TQ), F32),
            pltpu.VMEM((8, TQ), F32),
            pltpu.VMEM((2, VR, TQ), F32),
            pltpu.SemaphoreType.DMA((5,)),
            pltpu.SemaphoreType.DMA((3 + NC,)),
            pltpu.SemaphoreType.DMA((1,)),
        ],
        compiler_params=pltpu.CompilerParams(vmem_limit_bytes=110 * 1024 * 1024),
    )(A_x.reshape(NB, L, D), A_wqkv, A_wo, B_k.reshape(NB, L, D), B_v.reshape(NB, L, D),
      B_shift_k.T, B_ssm_k, B_ssm_D.reshape(NT, L), gate_w.reshape(NT, L))
    return out.reshape(1, S, D)
```

```python
import functools
import math

import jax
import jax.numpy as jnp
import jax.experimental.pallas as pl
import jax.experimental.pallas.tpu as pltpu

S = 2048
D = 640
H = 32
DH = D // H
KS = 4
L = 128
NT = D // L
NB = S // L
NG = L // 8
VR = 24
TQ = 512
TK = 128
NQB = S // TQ
NKB = S // TK
LAG = 3
CH = 512
NC = S // CH
CB = CH // L
QB = (NB - CB) // 2
RA = 2
TA = 3

F32 = jnp.float32
BF16 = jnp.bfloat16
U32 = jnp.uint32
_NT_DIMS = (((1,), (1,)), ((), ()))


def _head_geometry(h):
    lo, hi = DH * h, DH * h + DH - 1
    t0, t1 = lo // L, hi // L
    return t0, t1, lo - L * t0, hi + 1 - L * t1


def _pack(x):
    return pltpu.bitcast(x.astype(BF16), U32)


def _unpack(x):
    return pltpu.bitcast(x, BF16)


def _halves(w):
    return [jax.lax.bitcast_convert_type(w << 16, F32),
            jax.lax.bitcast_convert_type(w & jnp.uint32(0xFFFF0000), F32)]


def _pack_pair(lo, hi):
    def bits(x):
        return jax.lax.bitcast_convert_type(x.astype(BF16).astype(F32), U32)
    return (bits(lo) >> 16) | bits(hi)


def _dft_tables():
    def cos_table(k):
        k = k & (4 * L - 1)
        return jnp.cos(k.astype(F32) * (math.pi / (2 * L)))

    r = jax.lax.broadcasted_iota(jnp.int32, (2 * L, L), 0)
    n = jax.lax.broadcasted_iota(jnp.int32, (2 * L, L), 1)
    fr = r & (L - 1)
    f = jnp.where(fr < L // 2, 2 * fr, 2 * L - 1 - 2 * fr)
    fwd = cos_table((2 * f + 1) * n + jnp.where(r >= L, L, 0))
    a = jax.lax.broadcasted_iota(jnp.int32, (L, L), 0)
    c = jax.lax.broadcasted_iota(jnp.int32, (L, L), 1)
    t = jnp.where(a < L // 2, 2 * a, 2 * a - (L - 1))
    inv = cos_table((4 * (c >> 1) + 1) * t + (c & 1) * L) * (1.0 / L)
    return _pack(fwd), _pack(inv)


def _kernel(x_hbm, wqkv_hbm, wo_hbm, k_hbm, v_hbm, sk_hbm, h_hbm, sd_hbm, gw_hbm,
            o_hbm,
            x_ref, wqkv_ref, wo_ref, k_ref, v_ref, sk_ref, h_ref, sd_ref, gw_ref, o_ref,
            qm_ref, kt_ref, vt_ref, ot_ref, u_ref, hf_ref, hp_ref, z_ref, g_ref,
            fwd_ref, inv_ref, row_ref, cs_ref, cm_ref, ca_ref,
            wsem, csem, osem):
    def w_copy(i):
        cols = slice(i * D, (i + 1) * D)
        return pltpu.make_async_copy(wqkv_hbm.at[:, cols], wqkv_ref.at[:, cols], wsem.at[i])

    def wo_copy():
        return pltpu.make_async_copy(wo_hbm, wo_ref, wsem.at[3])

    def small_copies():
        return [pltpu.make_async_copy(sk_hbm, sk_ref, wsem.at[4]),
                pltpu.make_async_copy(sd_hbm, sd_ref, wsem.at[4]),
                pltpu.make_async_copy(gw_hbm, gw_ref, wsem.at[4])]

    def x_copy(c):
        blk = pl.ds(CB + (c - 1) * QB, QB)
        return pltpu.make_async_copy(x_hbm.at[blk], x_ref.at[blk], csem.at[c])

    def conv_copies(c):
        rows = pl.ds(pl.multiple_of(c * CH, CH), CH)
        blk = pl.ds(c * CB, CB)
        sem = csem.at[3 + c]
        return [pltpu.make_async_copy(k_hbm.at[blk], k_ref.at[pl.ds(c * CB + 1, CB)], sem),
                pltpu.make_async_copy(v_hbm.at[blk], v_ref.at[blk], sem),
                pltpu.make_async_copy(h_hbm.at[:, rows], h_ref.at[c], sem)]

    def out_copy(i, cols=slice(None)):
        rows = slice(i * L, (i + 1) * L)
        return pltpu.make_async_copy(o_ref.at[rows, cols], o_hbm.at[rows, cols], osem.at[0])

    def first_copies(part):
        blk = slice(0, RA) if part == 0 else slice(RA, CB)
        cols = slice(0, TA * L) if part == 0 else slice(TA * L, D)
        sem = wsem.at[0] if part == 0 else csem.at[0]
        return [pltpu.make_async_copy(x_hbm.at[blk], x_ref.at[blk], sem),
                pltpu.make_async_copy(wqkv_hbm.at[:, cols], wqkv_ref.at[:, cols], sem)]

    for cp in first_copies(0) + first_copies(1):
        cp.start()

    lane = jax.lax.broadcasted_iota(jnp.int32, (1, L), 1)
    row8 = jax.lax.broadcasted_iota(jnp.int32, (8, 1), 0)
    qscale = (DH ** -0.5) * math.log2(math.e)

    def chunk_rows(c):
        return (pl.ds(pl.multiple_of(c * CH, CH), CH),
                pl.ds(pl.multiple_of(c * (CH // 2), CH // 2), CH // 2))

    def x_rows(b0, nb):
        return x_ref[pl.ds(b0, nb)].reshape(nb * L, D)

    def proj_q(b0, nb, t_lo=0, t_hi=NT, qt=None):
        prows = pl.ds(pl.multiple_of(b0 * (L // 2), L // 2), nb * L // 2)
        q = jnp.dot(x_rows(b0, nb), wqkv_ref[:, t_lo * L:t_hi * L],
                    preferred_element_type=F32)
        qt = dict(qt or {})
        for t in range(t_lo, t_hi):
            qt[t] = _pack(q[:, (t - t_lo) * L:(t - t_lo + 1) * L] * qscale)
        zero = jnp.uint32(0)
        for h in range(H):
            t0, t1, lo, hi = _head_geometry(h)
            if not t_lo <= t1 < t_hi:
                continue
            if t0 == t1:
                qm = jnp.where((lane >= lo) & (lane < hi), qt[t0], zero)
            else:
                qm = jnp.where(lane >= lo, qt[t0], jnp.where(lane < hi, qt[t1], zero))
            qm_ref[h, prows, :] = qm
        return qt

    def proj_k(c):
        _, prows = chunk_rows(c)
        k = jnp.dot(x_rows(c * CB, CB), wqkv_ref[:, D:2 * D], preferred_element_type=F32)
        kt = [_pack(k[:, t * L:(t + 1) * L]) for t in range(NT)]
        for t in range(NT):
            kt_ref[t, prows, :] = kt[t]
        for t in range(NT - 1):
            kt_ref[NT + t, prows, :] = jnp.where(lane >= L // 2, kt[t], kt[t + 1])

    def proj_v(c):
        rows, _ = chunk_rows(c)
        v = jnp.dot(x_rows(c * CB, CB), wqkv_ref[:, 2 * D:3 * D], preferred_element_type=F32)
        vt = v.astype(BF16).astype(F32).T
        for p in range(H // 2):
            b = 2 * DH * p
            mid = vt[b + 16:b + 24]
            vt_ref[2 * p, 0:16, rows] = vt[b:b + 16]
            vt_ref[2 * p, 16:24, rows] = jnp.where(row8 == 4, 1.0, mid)
            vt_ref[2 * p + 1, 0:8, rows] = jnp.where(row8 == 0, 1.0, mid)
            vt_ref[2 * p + 1, 8:24, rows] = vt[b + 24:b + 40]

    def conv_u(c, s):
        j = c * CB + s
        for t in range(NT):
            cs = slice(t * L, (t + 1) * L)
            w = jnp.concatenate([pltpu.bitcast(k_ref[j, L - 16:L, cs], U32),
                                 pltpu.bitcast(k_ref[j + 1, :, cs], U32)], axis=0)
            e0, o0 = _halves(w[8:8 + L // 2])
            e1, o1 = _halves(pltpu.roll(w, 1, 0)[8:8 + L // 2])
            o2 = _halves(pltpu.roll(w, 2, 0)[8:8 + L // 2])[1]
            s0, s1, s2, s3 = [row_ref[d:d + 1, cs] for d in range(KS)]
            ve, vo = _halves(pltpu.bitcast(v_ref[j, :, cs], U32))
            kve = (e0 * s0 + o1 * s1 + e1 * s2 + o2 * s3) * ve
            kvo = (o0 * s0 + e0 * s1 + o1 * s2 + e1 * s3) * vo
            u = jnp.dot(_unpack(fwd_ref[...]), _unpack(_pack_pair(kve, kvo)),
                        preferred_element_type=F32)
            for r in range(2):
                u_ref[:, t, c, 2 * s + r] = u[r * L:(r + 1) * L].reshape(NG, 8, L)

    def conv_h(c, s, hp, skip):
        hc = jax.lax.dot_general(_unpack(fwd_ref[...]), h_ref[c, :, s * L:(s + 1) * L],
                                 _NT_DIMS, preferred_element_type=F32)
        if skip is not None:
            hc = jnp.concatenate([hc[0:L] + skip, hc[L:2 * L]], axis=0)
        hl = L // 2
        hf = jnp.concatenate([
            hc[0:hl] - hp[L:L + hl], hc[hl:L] + hp[L + hl:2 * L],
            hc[L:L + hl] + hp[0:hl], hc[L + hl:2 * L] - hp[hl:L]], axis=0)
        for t in range(NT):
            for r in range(2):
                hf_ref[:, t, c, 2 * s + r] = (
                    hf[r * L:(r + 1) * L, t * L:(t + 1) * L].reshape(NG, 8, L))
        return hc

    fwd_ref[...], inv_ref[...] = _dft_tables()
    hp_ref[...] = jnp.zeros(hp_ref.shape, F32)
    k_ref[0, L - 16:L, :] = jnp.zeros((16, D), BF16)
    cs_ref[...] = jnp.zeros(cs_ref.shape, F32)
    cm_ref[...] = jnp.zeros(cm_ref.shape, F32)
    ca_ref[...] = jnp.ones(ca_ref.shape, F32)

    for cp in first_copies(0):
        cp.wait()
    x_copy(1).start()
    qt = [proj_q(b, 1, 0, TA) for b in range(RA)]
    for cp in first_copies(1):
        cp.wait()
    x_copy(2).start()
    proj_q(RA, CB - RA)
    for b in range(RA):
        proj_q(b, 1, TA, NT, qt[b])

    def qpass(c, carry):
        x_copy(c).wait()

        @pl.when(c == 1)
        def _():
            for cp in small_copies() + [w_copy(1), w_copy(2)] + conv_copies(0):
                cp.start()

        proj_q(CB + (c - 1) * QB, QB)
        return carry

    jax.lax.fori_loop(1, 3, qpass, 0)
    for c in range(1, NC):
        for cp in conv_copies(c):
            cp.start()
    wo_copy().start()
    w_copy(1).wait()
    w_copy(2).wait()
    for cp in small_copies():
        cp.wait()
    row_ref[0:KS, :] = sk_ref[...].astype(F32)
    for t in range(NT):
        row_ref[KS:KS + 1, t * L:(t + 1) * L] = sd_ref[...].astype(F32)[t:t + 1]
        row_ref[KS + 1:KS + 2, t * L:(t + 1) * L] = gw_ref[...].astype(F32)[t:t + 1]

    def kvpass(c, carry):
        for cp in conv_copies(c):
            cp.wait()
        proj_v(c)
        hp = hp_ref[...]
        for s in range(CB):
            skip = jnp.where(c == 0, row_ref[KS:KS + 1, :], 0.0) if s == 0 else None
            hp = conv_h(c, s, hp, skip)
            conv_u(c, s)
        hp_ref[...] = hp
        proj_k(c)
        return carry

    jax.lax.fori_loop(0, NC, kvpass, 0)
    wo_copy().wait()

    def ktile(h):
        lo = h * DH
        t0 = lo // L
        return t0 + NT * ((lo - t0 * L) > (L - DH)).astype(jnp.int32)

    def attention(p, flush_only=False):
        heads = {0: 2 * p, 1: 2 * p + 1,
                 -1: H - 1 if flush_only else jnp.maximum(2 * p - 1, 0)}
        blocks = [(-1, NQB - 1, kb) for kb in range(NKB - LAG, NKB)]
        if not flush_only:
            kidx = [ktile(heads[e]) for e in range(2)]
            blocks += [(e, qi, kb) for qi in range(NQB) for e in range(2)
                       for kb in range(NKB)]
        ss = {blocks[n]: cs_ref[n] for n in range(LAG)}
        ms = {(-1, NQB - 1): cm_ref[0:1]}
        accs = {(-1, NQB - 1): ca_ref[0]}
        outs = {(-2, NQB - 1): ca_ref[1]}

        def qk(e, qi, kb):
            q = _unpack(qm_ref[heads[e], qi * TQ // 2:(qi + 1) * TQ // 2, :])
            kk = _unpack(kt_ref[kidx[e], kb * TK // 2:(kb + 1) * TK // 2, :])
            ss[(e, qi, kb)] = jax.lax.dot_general(kk, q, _NT_DIMS,
                                                  preferred_element_type=F32)

        def softmax_pv(e, qi, kb):
            st = ss.pop((e, qi, kb))
            mn = jnp.max(st, axis=0, keepdims=True)
            if kb > 0:
                mn = jnp.maximum(ms[(e, qi)], mn)
                alpha = jnp.exp2(ms[(e, qi)] - mn)
            ms[(e, qi)] = mn
            pt = jnp.exp2(st - mn).astype(BF16)
            r = jnp.dot(vt_ref[heads[e], :, kb * TK:(kb + 1) * TK], pt,
                        preferred_element_type=F32)
            accs[(e, qi)] = r if kb == 0 else accs[(e, qi)] * alpha + r
            if kb == NKB - 1:
                acc = accs.pop((e, qi))
                den = acc[20:21] if e % 2 == 0 else acc[0:1]
                outs[(e, qi)] = acc * (1.0 / den)
                if e % 2 == 1:
                    oe, oo = outs.pop((e - 1, qi)), outs.pop((e, qi))
                    cols = slice(qi * TQ, (qi + 1) * TQ)
                    slot = p + e // 2 + 1
                    ot_ref[slot, 0:16, cols] = oe[0:16]
                    ot_ref[slot, 16:24, cols] = jnp.where(row8 < 4, oe[16:24], oo[0:8])
                    ot_ref[slot, 24:40, cols] = oo[8:24]

        if flush_only:
            return [functools.partial(softmax_pv, *b) for b in blocks]

        zacc = {}
        pz = p & (NG // 2 - 1)
        pq = p ^ (NG // 2)

        def at(g, t, j, r):
            return (g, t, j // CB, 2 * (j % CB) + r)

        def conv_step(t, m, zero):
            hr, hi_ = hf_ref[at(p, t, m, 0)] + zero, hf_ref[at(p, t, m, 1)] + zero
            for i in range(m, NB):
                ur, ui = u_ref[at(p, t, i - m, 0)], u_ref[at(p, t, i - m, 1)]
                tr = ur * hr - ui * hi_
                ti = ur * hi_ + ui * hr
                if m > 0:
                    tr, ti = zacc[i][0] + tr, zacc[i][1] + ti
                zacc[i] = (tr, ti)
                if m == i:
                    wr, wi = hf_ref[at(pq, t, i, 0)], hf_ref[at(pq, t, i, 1)]
                    hf_ref[at(p, t, i, 0)] = tr
                    hf_ref[at(p, t, i, 1)] = ti
                    z_ref[pz, i, 0, t] = _pack_pair(wr + tr, wi - ti)
                    z_ref[pz, i, 1, t] = _pack_pair(wr - tr, wi + ti)

        steps = [(t, m) for t in range(NT) for m in range(NB)]
        nb = len(blocks) - LAG
        hosts = [n for n in range(nb) if blocks[n][2] not in (0, NKB - 1)]
        slot_of = [hosts[k * len(hosts) // len(steps)] for k in range(len(steps))]
        for n in range(nb):
            qk(*blocks[n + LAG])
            softmax_pv(*blocks[n])
            zero = jnp.where(ss[blocks[n + 1]][0:8, 0:L] > 0, 0.0, -0.0)
            for step, host in zip(steps, slot_of):
                if host == n:
                    conv_step(*step, zero)
        rows = pl.ds(pl.multiple_of(p * L, L), L)
        logit = jnp.sum(x_ref[p].astype(F32) * row_ref[KS + 1:KS + 2, :],
                        axis=-1, keepdims=True)
        g_ref[rows, :] = jnp.broadcast_to(jax.nn.sigmoid(logit), (L, L))
        for n in range(LAG):
            cs_ref[n] = ss.pop(blocks[nb + n])
        cm_ref[0:1] = ms[(1, NQB - 1)]
        ca_ref[0] = accs.pop((1, NQB - 1))
        ca_ref[1] = outs.pop((0, NQB - 1))

    def pair(p, carry):
        attention(p)
        return carry

    jax.lax.fori_loop(0, H // 2, pair, 0)

    lane_tiles = [slice(t * L, (t + 1) * L) for t in range(NT)]
    flush = attention(H // 2, flush_only=True)
    for i in range(NB):
        rows = slice(i * L, (i + 1) * L)
        yh = []
        for e in range(2):
            w = jnp.concatenate(
                [_unpack(z_ref[:, i, e, t].reshape(L // 2, L)) for t in range(NT)], axis=1)
            yh.append(jnp.dot(_unpack(inv_ref[e * L // 4:(e + 1) * L // 4, :]), w,
                              preferred_element_type=F32))
        y = _unpack(_pack_pair(*yh)).astype(F32)
        b = (jnp.concatenate([1.0 - g_ref[rows, :]] * NT, axis=1)
             * (x_ref[i].astype(F32) * y))
        ot = ot_ref[1:, :, rows].reshape(D, L)
        a = jnp.dot(ot.T.astype(BF16), wo_ref[...], preferred_element_type=F32)
        g = jnp.concatenate([g_ref[rows, :]] * NT, axis=1)
        out = (g * a + b).astype(o_ref.dtype)
        for cols in ([slice(None)] if i < NB - 1 else lane_tiles):
            o_ref[rows, cols] = out[:, cols]
            out_copy(i, cols).start()
        if i < LAG:
            flush[i]()
    for i in range(NB - 1):
        out_copy(i).wait()
    for cols in lane_tiles:
        out_copy(NB - 1, cols).wait()


@jax.jit
def pallas_gated_mix__mha_block__ssm_conv_h3__prompt_kernel(
    A_x: jax.Array,
    A_wqkv: jax.Array,
    A_wo: jax.Array,
    B_q: jax.Array,
    B_k: jax.Array,
    B_v: jax.Array,
    B_shift_k: jax.Array,
    B_ssm_k: jax.Array,
    B_ssm_D: jax.Array,
    gate_w: jax.Array,
):
    del B_q
    out = pl.pallas_call(
        _kernel,
        out_shape=jax.ShapeDtypeStruct((S, D), BF16),
        in_specs=[pl.BlockSpec(memory_space=pl.ANY)] * 9,
        out_specs=pl.BlockSpec(memory_space=pl.ANY),
        scratch_shapes=[
            pltpu.VMEM((NB, L, D), BF16),
            pltpu.VMEM((D, 3 * D), BF16),
            pltpu.VMEM((D, D), BF16),
            pltpu.VMEM((NB + 1, L, D), BF16),
            pltpu.VMEM((NB, L, D), BF16),
            pltpu.VMEM((KS, D), BF16),
            pltpu.VMEM((NC, D, CH), BF16),
            pltpu.VMEM((NT, L), BF16),
            pltpu.VMEM((NT, L), BF16),
            pltpu.VMEM((S, D), BF16),
            pltpu.VMEM((H, S // 2, L), U32),
            pltpu.VMEM((2 * NT - 1, S // 2, L), U32),
            pltpu.VMEM((H, VR, S), F32),
            pltpu.VMEM((H // 2 + 1, 2 * DH, S), F32),
            pltpu.VMEM((NG, NT, NC, 2 * CB, 8, L), F32),
            pltpu.VMEM((NG, NT, NC, 2 * CB, 8, L), F32),
            pltpu.VMEM((2 * L, D), F32),
            pltpu.VMEM((NG // 2, NB, 2, NT, 8, L), U32),
            pltpu.VMEM((S, L), F32),
            pltpu.VMEM((L, L), U32),
            pltpu.VMEM((L // 2, L), U32),
            pltpu.VMEM((8, D), F32),
            pltpu.VMEM((LAG, TK, TQ), F32),
            pltpu.VMEM((8, TQ), F32),
            pltpu.VMEM((2, VR, TQ), F32),
            pltpu.SemaphoreType.DMA((5,)),
            pltpu.SemaphoreType.DMA((3 + NC,)),
            pltpu.SemaphoreType.DMA((1,)),
        ],
        compiler_params=pltpu.CompilerParams(vmem_limit_bytes=110 * 1024 * 1024),
    )(A_x.reshape(NB, L, D), A_wqkv, A_wo, B_k.reshape(NB, L, D), B_v.reshape(NB, L, D),
      B_shift_k.T, B_ssm_k, B_ssm_D.reshape(NT, L), gate_w.reshape(NT, L))
    return out.reshape(1, S, D)
```

```python
import functools
import math

import jax
import jax.numpy as jnp
import jax.experimental.pallas as pl
import jax.experimental.pallas.tpu as pltpu

S = 2048
D = 640
H = 32
DH = D // H
KS = 4
L = 128
NT = D // L
NB = S // L
NG = L // 8
VR = 24
TQ = 512
TK = 128
NQB = S // TQ
NKB = S // TK
LAG = 3
CH = 512
NC = S // CH
CB = CH // L
QB = (NB - CB) // 2
RA = 2
TA = 3

F32 = jnp.float32
BF16 = jnp.bfloat16
U32 = jnp.uint32
_NT_DIMS = (((1,), (1,)), ((), ()))


def _head_geometry(h):
    lo, hi = DH * h, DH * h + DH - 1
    t0, t1 = lo // L, hi // L
    return t0, t1, lo - L * t0, hi + 1 - L * t1


def _pack(x):
    return pltpu.bitcast(x.astype(BF16), U32)


def _unpack(x):
    return pltpu.bitcast(x, BF16)


def _halves(w):
    return [jax.lax.bitcast_convert_type(w << 16, F32),
            jax.lax.bitcast_convert_type(w & jnp.uint32(0xFFFF0000), F32)]


def _pack_pair(lo, hi):
    def bits(x):
        return jax.lax.bitcast_convert_type(x.astype(BF16).astype(F32), U32)
    return (bits(lo) >> 16) | bits(hi)


def _dft_tables():
    def cos_table(k):
        k = k & (4 * L - 1)
        return jnp.cos(k.astype(F32) * (math.pi / (2 * L)))

    r = jax.lax.broadcasted_iota(jnp.int32, (2 * L, L), 0)
    n = jax.lax.broadcasted_iota(jnp.int32, (2 * L, L), 1)
    fr = r & (L - 1)
    f = jnp.where(fr < L // 2, 2 * fr, 2 * L - 1 - 2 * fr)
    fwd = cos_table((2 * f + 1) * n + jnp.where(r >= L, L, 0))
    a = jax.lax.broadcasted_iota(jnp.int32, (L, L), 0)
    c = jax.lax.broadcasted_iota(jnp.int32, (L, L), 1)
    t = jnp.where(a < L // 2, 2 * a, 2 * a - (L - 1))
    inv = cos_table((4 * (c >> 1) + 1) * t + (c & 1) * L) * (1.0 / L)
    return _pack(fwd), _pack(inv)


def _kernel(x_hbm, wqkv_hbm, wo_hbm, k_hbm, v_hbm, sk_hbm, h_hbm, sd_hbm, gw_hbm,
            o_hbm,
            x_ref, wqkv_ref, wo_ref, k_ref, v_ref, sk_ref, h_ref, sd_ref, gw_ref, o_ref,
            qm_ref, kt_ref, vt_ref, ot_ref, u_ref, hf_ref, hp_ref, z_ref, g_ref,
            fwd_ref, inv_ref, row_ref, cs_ref, cm_ref, ca_ref,
            wsem, csem, osem):
    def w_copy(i):
        cols = slice(i * D, (i + 1) * D)
        return pltpu.make_async_copy(wqkv_hbm.at[:, cols], wqkv_ref.at[:, cols], wsem.at[i])

    def wo_copy():
        return pltpu.make_async_copy(wo_hbm, wo_ref, wsem.at[3])

    def small_copies():
        return [pltpu.make_async_copy(sk_hbm, sk_ref, wsem.at[4]),
                pltpu.make_async_copy(sd_hbm, sd_ref, wsem.at[4]),
                pltpu.make_async_copy(gw_hbm, gw_ref, wsem.at[4])]

    def x_copy(c):
        blk = pl.ds(CB + (c - 1) * QB, QB)
        return pltpu.make_async_copy(x_hbm.at[blk], x_ref.at[blk], csem.at[c])

    def conv_copies(c):
        rows = pl.ds(pl.multiple_of(c * CH, CH), CH)
        blk = pl.ds(c * CB, CB)
        sem = csem.at[3 + c]
        return [pltpu.make_async_copy(k_hbm.at[blk], k_ref.at[pl.ds(c * CB + 1, CB)], sem),
                pltpu.make_async_copy(v_hbm.at[blk], v_ref.at[blk], sem),
                pltpu.make_async_copy(h_hbm.at[:, rows], h_ref.at[c], sem)]

    def out_copy(i, cols=slice(None)):
        rows = slice(i * L, (i + 1) * L)
        return pltpu.make_async_copy(o_ref.at[rows, cols], o_hbm.at[rows, cols], osem.at[0])

    def first_copies(part):
        blk = slice(0, RA) if part == 0 else slice(RA, CB)
        cols = slice(0, TA * L) if part == 0 else slice(TA * L, D)
        sem = wsem.at[0] if part == 0 else csem.at[0]
        return [pltpu.make_async_copy(x_hbm.at[blk], x_ref.at[blk], sem),
                pltpu.make_async_copy(wqkv_hbm.at[:, cols], wqkv_ref.at[:, cols], sem)]

    for cp in first_copies(0) + first_copies(1):
        cp.start()

    lane = jax.lax.broadcasted_iota(jnp.int32, (1, L), 1)
    row8 = jax.lax.broadcasted_iota(jnp.int32, (8, 1), 0)
    qscale = (DH ** -0.5) * math.log2(math.e)

    def chunk_rows(c):
        return (pl.ds(pl.multiple_of(c * CH, CH), CH),
                pl.ds(pl.multiple_of(c * (CH // 2), CH // 2), CH // 2))

    def x_rows(b0, nb):
        return x_ref[pl.ds(b0, nb)].reshape(nb * L, D)

    def proj_q(b0, nb, t_lo=0, t_hi=NT, qt=None):
        prows = pl.ds(pl.multiple_of(b0 * (L // 2), L // 2), nb * L // 2)
        q = jnp.dot(x_rows(b0, nb), wqkv_ref[:, t_lo * L:t_hi * L],
                    preferred_element_type=F32)
        qt = dict(qt or {})
        for t in range(t_lo, t_hi):
            qt[t] = _pack(q[:, (t - t_lo) * L:(t - t_lo + 1) * L] * qscale)
        zero = jnp.uint32(0)
        for h in range(H):
            t0, t1, lo, hi = _head_geometry(h)
            if not t_lo <= t1 < t_hi:
                continue
            if t0 == t1:
                qm = jnp.where((lane >= lo) & (lane < hi), qt[t0], zero)
            else:
                qm = jnp.where(lane >= lo, qt[t0], jnp.where(lane < hi, qt[t1], zero))
            qm_ref[h, prows, :] = qm
        return qt

    def proj_k(c):
        _, prows = chunk_rows(c)
        k = jnp.dot(x_rows(c * CB, CB), wqkv_ref[:, D:2 * D], preferred_element_type=F32)
        kt = [_pack(k[:, t * L:(t + 1) * L]) for t in range(NT)]
        for t in range(NT):
            kt_ref[t, prows, :] = kt[t]
        for t in range(NT - 1):
            kt_ref[NT + t, prows, :] = jnp.where(lane >= L // 2, kt[t], kt[t + 1])

    def proj_v(c):
        rows, _ = chunk_rows(c)
        v = jnp.dot(x_rows(c * CB, CB), wqkv_ref[:, 2 * D:3 * D], preferred_element_type=F32)
        vt = v.astype(BF16).astype(F32).T
        for p in range(H // 2):
            b = 2 * DH * p
            mid = vt[b + 16:b + 24]
            vt_ref[2 * p, 0:16, rows] = vt[b:b + 16]
            vt_ref[2 * p, 16:24, rows] = jnp.where(row8 == 4, 1.0, mid)
            vt_ref[2 * p + 1, 0:8, rows] = jnp.where(row8 == 0, 1.0, mid)
            vt_ref[2 * p + 1, 8:24, rows] = vt[b + 24:b + 40]

    def conv_u(c, s):
        j = c * CB + s
        for t in range(NT):
            cs = slice(t * L, (t + 1) * L)
            w = jnp.concatenate([pltpu.bitcast(k_ref[j, L - 16:L, cs], U32),
                                 pltpu.bitcast(k_ref[j + 1, :, cs], U32)], axis=0)
            e0, o0 = _halves(w[8:8 + L // 2])
            e1, o1 = _halves(pltpu.roll(w, 1, 0)[8:8 + L // 2])
            o2 = _halves(pltpu.roll(w, 2, 0)[8:8 + L // 2])[1]
            s0, s1, s2, s3 = [row_ref[d:d + 1, cs] for d in range(KS)]
            ve, vo = _halves(pltpu.bitcast(v_ref[j, :, cs], U32))
            kve = (e0 * s0 + o1 * s1 + e1 * s2 + o2 * s3) * ve
            kvo = (o0 * s0 + e0 * s1 + o1 * s2 + e1 * s3) * vo
            u = jnp.dot(_unpack(fwd_ref[...]), _unpack(_pack_pair(kve, kvo)),
                        preferred_element_type=F32)
            for r in range(2):
                u_ref[:, t, c, 2 * s + r] = u[r * L:(r + 1) * L].reshape(NG, 8, L)

    def conv_h(c, s, hp, skip):
        hc = jax.lax.dot_general(_unpack(fwd_ref[...]), h_ref[c, :, s * L:(s + 1) * L],
                                 _NT_DIMS, preferred_element_type=F32)
        if skip is not None:
            hc = jnp.concatenate([hc[0:L] + skip, hc[L:2 * L]], axis=0)
        hl = L // 2
        hf = jnp.concatenate([
            hc[0:hl] - hp[L:L + hl], hc[hl:L] + hp[L + hl:2 * L],
            hc[L:L + hl] + hp[0:hl], hc[L + hl:2 * L] - hp[hl:L]], axis=0)
        for t in range(NT):
            for r in range(2):
                hf_ref[:, t, c, 2 * s + r] = (
                    hf[r * L:(r + 1) * L, t * L:(t + 1) * L].reshape(NG, 8, L))
        return hc

    fwd_ref[...], inv_ref[...] = _dft_tables()
    hp_ref[...] = jnp.zeros(hp_ref.shape, F32)
    k_ref[0, L - 16:L, :] = jnp.zeros((16, D), BF16)
    cs_ref[...] = jnp.zeros(cs_ref.shape, F32)
    cm_ref[...] = jnp.zeros(cm_ref.shape, F32)
    ca_ref[...] = jnp.ones(ca_ref.shape, F32)

    for cp in first_copies(0):
        cp.wait()
    x_copy(1).start()
    qt = [proj_q(b, 1, 0, TA) for b in range(RA)]
    for cp in first_copies(1):
        cp.wait()
    x_copy(2).start()
    proj_q(RA, CB - RA)
    for b in range(RA):
        proj_q(b, 1, TA, NT, qt[b])

    for cp in small_copies() + [w_copy(1), w_copy(2)] + conv_copies(0):
        cp.start()

    def qpass(c, carry):
        x_copy(c).wait()
        proj_q(CB + (c - 1) * QB, QB)
        return carry

    jax.lax.fori_loop(1, 3, qpass, 0)
    for c in range(1, NC):
        for cp in conv_copies(c):
            cp.start()
    wo_copy().start()
    w_copy(1).wait()
    w_copy(2).wait()
    for cp in small_copies():
        cp.wait()
    row_ref[0:KS, :] = sk_ref[...].astype(F32)
    for t in range(NT):
        row_ref[KS:KS + 1, t * L:(t + 1) * L] = sd_ref[...].astype(F32)[t:t + 1]
        row_ref[KS + 1:KS + 2, t * L:(t + 1) * L] = gw_ref[...].astype(F32)[t:t + 1]

    def kvpass(c, carry):
        for cp in conv_copies(c):
            cp.wait()
        proj_v(c)
        hp = hp_ref[...]
        for s in range(CB):
            skip = jnp.where(c == 0, row_ref[KS:KS + 1, :], 0.0) if s == 0 else None
            hp = conv_h(c, s, hp, skip)
            conv_u(c, s)
        hp_ref[...] = hp
        proj_k(c)
        return carry

    jax.lax.fori_loop(0, NC, kvpass, 0)
    wo_copy().wait()

    def ktile(h):
        lo = h * DH
        t0 = lo // L
        return t0 + NT * ((lo - t0 * L) > (L - DH)).astype(jnp.int32)

    def attention(p, flush_only=False):
        heads = {0: 2 * p, 1: 2 * p + 1,
                 -1: H - 1 if flush_only else jnp.maximum(2 * p - 1, 0)}
        blocks = [(-1, NQB - 1, kb) for kb in range(NKB - LAG, NKB)]
        if not flush_only:
            kidx = [ktile(heads[e]) for e in range(2)]
            blocks += [(e, qi, kb) for qi in range(NQB) for e in range(2)
                       for kb in range(NKB)]
        ss = {blocks[n]: cs_ref[n] for n in range(LAG)}
        ms = {(-1, NQB - 1): cm_ref[0:1]}
        accs = {(-1, NQB - 1): ca_ref[0]}
        outs = {(-2, NQB - 1): ca_ref[1]}

        def qk(e, qi, kb):
            q = _unpack(qm_ref[heads[e], qi * TQ // 2:(qi + 1) * TQ // 2, :])
            kk = _unpack(kt_ref[kidx[e], kb * TK // 2:(kb + 1) * TK // 2, :])
            ss[(e, qi, kb)] = jax.lax.dot_general(kk, q, _NT_DIMS,
                                                  preferred_element_type=F32)

        def softmax_pv(e, qi, kb):
            st = ss.pop((e, qi, kb))
            mn = jnp.max(st, axis=0, keepdims=True)
            if kb > 0:
                mn = jnp.maximum(ms[(e, qi)], mn)
                alpha = jnp.exp2(ms[(e, qi)] - mn)
            ms[(e, qi)] = mn
            pt = jnp.exp2(st - mn).astype(BF16)
            r = jnp.dot(vt_ref[heads[e], :, kb * TK:(kb + 1) * TK], pt,
                        preferred_element_type=F32)
            accs[(e, qi)] = r if kb == 0 else accs[(e, qi)] * alpha + r
            if kb == NKB - 1:
                acc = accs.pop((e, qi))
                den = acc[20:21] if e % 2 == 0 else acc[0:1]
                outs[(e, qi)] = acc * (1.0 / den)
                if e % 2 == 1:
                    oe, oo = outs.pop((e - 1, qi)), outs.pop((e, qi))
                    cols = slice(qi * TQ, (qi + 1) * TQ)
                    slot = p + e // 2 + 1
                    ot_ref[slot, 0:16, cols] = oe[0:16]
                    ot_ref[slot, 16:24, cols] = jnp.where(row8 < 4, oe[16:24], oo[0:8])
                    ot_ref[slot, 24:40, cols] = oo[8:24]

        if flush_only:
            return [functools.partial(softmax_pv, *b) for b in blocks]

        zacc = {}
        pz = p & (NG // 2 - 1)
        pq = p ^ (NG // 2)

        def at(g, t, j, r):
            return (g, t, j // CB, 2 * (j % CB) + r)

        def conv_step(t, m, zero):
            hr, hi_ = hf_ref[at(p, t, m, 0)] + zero, hf_ref[at(p, t, m, 1)] + zero
            for i in range(m, NB):
                ur, ui = u_ref[at(p, t, i - m, 0)], u_ref[at(p, t, i - m, 1)]
                tr = ur * hr - ui * hi_
                ti = ur * hi_ + ui * hr
                if m > 0:
                    tr, ti = zacc[i][0] + tr, zacc[i][1] + ti
                zacc[i] = (tr, ti)
                if m == i:
                    wr, wi = hf_ref[at(pq, t, i, 0)], hf_ref[at(pq, t, i, 1)]
                    hf_ref[at(p, t, i, 0)] = tr
                    hf_ref[at(p, t, i, 1)] = ti
                    z_ref[pz, i, 0, t] = _pack_pair(wr + tr, wi - ti)
                    z_ref[pz, i, 1, t] = _pack_pair(wr - tr, wi + ti)

        steps = [(t, m) for t in range(NT) for m in range(NB)]
        nb = len(blocks) - LAG
        hosts = [n for n in range(nb) if blocks[n][2] not in (0, NKB - 1)]
        slot_of = [hosts[k * len(hosts) // len(steps)] for k in range(len(steps))]
        for n in range(nb):
            qk(*blocks[n + LAG])
            softmax_pv(*blocks[n])
            zero = jnp.where(ss[blocks[n + 1]][0:8, 0:L] > 0, 0.0, -0.0)
            for step, host in zip(steps, slot_of):
                if host == n:
                    conv_step(*step, zero)
        rows = pl.ds(pl.multiple_of(p * L, L), L)
        logit = jnp.sum(x_ref[p].astype(F32) * row_ref[KS + 1:KS + 2, :],
                        axis=-1, keepdims=True)
        g_ref[rows, :] = jnp.broadcast_to(jax.nn.sigmoid(logit), (L, L))
        for n in range(LAG):
            cs_ref[n] = ss.pop(blocks[nb + n])
        cm_ref[0:1] = ms[(1, NQB - 1)]
        ca_ref[0] = accs.pop((1, NQB - 1))
        ca_ref[1] = outs.pop((0, NQB - 1))

    def pair(p, carry):
        attention(p)
        return carry

    jax.lax.fori_loop(0, H // 2, pair, 0)

    lane_tiles = [slice(t * L, (t + 1) * L) for t in range(NT)]
    flush = attention(H // 2, flush_only=True)
    for i in range(NB):
        rows = slice(i * L, (i + 1) * L)
        yh = []
        for e in range(2):
            w = jnp.concatenate(
                [_unpack(z_ref[:, i, e, t].reshape(L // 2, L)) for t in range(NT)], axis=1)
            yh.append(jnp.dot(_unpack(inv_ref[e * L // 4:(e + 1) * L // 4, :]), w,
                              preferred_element_type=F32))
        y = _unpack(_pack_pair(*yh)).astype(F32)
        b = (jnp.concatenate([1.0 - g_ref[rows, :]] * NT, axis=1)
             * (x_ref[i].astype(F32) * y))
        ot = ot_ref[1:, :, rows].reshape(D, L)
        a = jnp.dot(ot.T.astype(BF16), wo_ref[...], preferred_element_type=F32)
        g = jnp.concatenate([g_ref[rows, :]] * NT, axis=1)
        out = (g * a + b).astype(o_ref.dtype)
        for cols in ([slice(None)] if i < NB - 1 else lane_tiles):
            o_ref[rows, cols] = out[:, cols]
            out_copy(i, cols).start()
        if i < LAG:
            flush[i]()
    for i in range(NB - 1):
        out_copy(i).wait()
    for cols in lane_tiles:
        out_copy(NB - 1, cols).wait()


@jax.jit
def pallas_gated_mix__mha_block__ssm_conv_h3__prompt_kernel(
    A_x: jax.Array,
    A_wqkv: jax.Array,
    A_wo: jax.Array,
    B_q: jax.Array,
    B_k: jax.Array,
    B_v: jax.Array,
    B_shift_k: jax.Array,
    B_ssm_k: jax.Array,
    B_ssm_D: jax.Array,
    gate_w: jax.Array,
):
    del B_q
    out = pl.pallas_call(
        _kernel,
        out_shape=jax.ShapeDtypeStruct((S, D), BF16),
        in_specs=[pl.BlockSpec(memory_space=pl.ANY)] * 9,
        out_specs=pl.BlockSpec(memory_space=pl.ANY),
        scratch_shapes=[
            pltpu.VMEM((NB, L, D), BF16),
            pltpu.VMEM((D, 3 * D), BF16),
            pltpu.VMEM((D, D), BF16),
            pltpu.VMEM((NB + 1, L, D), BF16),
            pltpu.VMEM((NB, L, D), BF16),
            pltpu.VMEM((KS, D), BF16),
            pltpu.VMEM((NC, D, CH), BF16),
            pltpu.VMEM((NT, L), BF16),
            pltpu.VMEM((NT, L), BF16),
            pltpu.VMEM((S, D), BF16),
            pltpu.VMEM((H, S // 2, L), U32),
            pltpu.VMEM((2 * NT - 1, S // 2, L), U32),
            pltpu.VMEM((H, VR, S), F32),
            pltpu.VMEM((H // 2 + 1, 2 * DH, S), F32),
            pltpu.VMEM((NG, NT, NC, 2 * CB, 8, L), F32),
            pltpu.VMEM((NG, NT, NC, 2 * CB, 8, L), F32),
            pltpu.VMEM((2 * L, D), F32),
            pltpu.VMEM((NG // 2, NB, 2, NT, 8, L), U32),
            pltpu.VMEM((S, L), F32),
            pltpu.VMEM((L, L), U32),
            pltpu.VMEM((L // 2, L), U32),
            pltpu.VMEM((8, D), F32),
            pltpu.VMEM((LAG, TK, TQ), F32),
            pltpu.VMEM((8, TQ), F32),
            pltpu.VMEM((2, VR, TQ), F32),
            pltpu.SemaphoreType.DMA((5,)),
            pltpu.SemaphoreType.DMA((3 + NC,)),
            pltpu.SemaphoreType.DMA((1,)),
        ],
        compiler_params=pltpu.CompilerParams(vmem_limit_bytes=110 * 1024 * 1024),
    )(A_x.reshape(NB, L, D), A_wqkv, A_wo, B_k.reshape(NB, L, D), B_v.reshape(NB, L, D),
      B_shift_k.T, B_ssm_k, B_ssm_D.reshape(NT, L), gate_w.reshape(NT, L))
    return out.reshape(1, S, D)
```
